```python
import os as _os
_os.environ.setdefault("JAX_PLATFORMS", "cpu")
import jax
import jax.numpy as jnp

def _softmax(x, axis=-1):
    return jax.nn.softmax(x, axis=axis)
def _gelu(x):
    return jax.nn.gelu(x, approximate=True)
def _silu(x):
    return jax.nn.silu(x)
def _sigmoid(x):
    return jax.nn.sigmoid(x)
def _layernorm(x, axis=-1, eps=1e-5):
    m = jnp.mean(x, axis=axis, keepdims=True)
    v = jnp.var(x, axis=axis, keepdims=True)
    return (x - m) / jnp.sqrt(v + eps)
def _scatter_add(tgt, idx, src, axis=0):
    return tgt.at[idx].add(src)
def _segment_sum(src, seg, n):
    return jax.ops.segment_sum(src, seg, n)
class _Rng:
    def __init__(self, key):
        self._k = key
    def _next(self):
        self._k, sub = jax.random.split(self._k)
        return sub
    def normal(self, shape):
        return jax.random.normal(self._next(), shape, dtype=jnp.bfloat16)
    def randint(self, lo, hi, shape):
        return jax.random.randint(self._next(), shape, lo, hi, dtype=jnp.int32)
    def uniform(self, shape, lo=0.0, hi=1.0):
        return jax.random.uniform(self._next(), shape, jnp.bfloat16, lo, hi)
    def permutation(self, n):
        return jax.random.permutation(self._next(), n)


kernel_name = 'standalone__detection_seg_fpn_lateral__vision'

def setup_inputs():
    _rng = _Rng(jax.random.key(int.from_bytes(__import__("os").urandom(4), "little")))
    _w = (lambda a: (lambda t: t.astype(jnp.bfloat16) if jnp.issubdtype(t.dtype, jnp.floating) else t)(jnp.asarray(a)))
    H = W = (256 // 2) * 2
    C = 384
    k = 1
    return {
        "c_fine": _w((lambda *s: _rng.normal(s) * 0.05)(1, H, W, C)),
        "p_coarse": _w((lambda *s: _rng.normal(s) * 0.05)(1, H // 2, W // 2, C)),
        "w_lat": _w((lambda *s: _rng.normal(s) * 0.05)(C, C)),
        "w_out": _w((lambda *s: _rng.normal(s) * 0.05)(k, k, C, C)),
    }

def reference(c_fine, p_coarse, w_lat, w_out):
    B, H, W, C = c_fine.shape
    k = 1
    lat = jnp.einsum("bhwc,cd->bhwd", c_fine, w_lat)
    up = jnp.repeat(jnp.repeat(p_coarse, 2, axis=1), 2, axis=2)
    m = lat + up
    pad = k // 2
    mp = jnp.pad(m, ((0, 0), (pad, pad), (pad, pad), (0, 0)))
    o = None
    for di in range(k):
        for dj in range(k):
            t = jnp.einsum("bhwc,cd->bhwd", mp[:, di:di + H, dj:dj + W, :], w_out[di, dj])
            o = t if o is None else o + t
    return o
```

```python
import jax
import jax.numpy as jnp
import jax.experimental.pallas as pl
import jax.experimental.pallas.tpu as pltpu

_TH = 4


def _kernel(c_ref, p_ref, wl_ref, wo_ref, o_ref, weff_ref):
    @pl.when(pl.program_id(0) == 0)
    def _():
        weff_ref[...] = jnp.dot(
            wl_ref[...], wo_ref[...], preferred_element_type=jnp.float32
        ).astype(weff_ref.dtype)

    wo = wo_ref[...]
    we = weff_ref[...]
    for r in range(_TH):
        q = jnp.dot(p_ref[r], wo, preferred_element_type=jnp.float32)
        qb = pltpu.bitcast(q.astype(jnp.bfloat16).astype(jnp.float32), jnp.uint32)
        up = pltpu.bitcast(qb | (qb >> 16), jnp.bfloat16).astype(jnp.float32)
        for hh in range(2):
            a = jnp.dot(c_ref[2 * r + hh], we, preferred_element_type=jnp.float32)
            o_ref[2 * r + hh] = (a + up).astype(o_ref.dtype)


@jax.jit
def pallas_standalone__detection_seg_fpn_lateral__vision_kernel(
    c_fine: jax.Array,
    p_coarse: jax.Array,
    w_lat: jax.Array,
    w_out: jax.Array,
):
    B, H, W, C = c_fine.shape
    out = pl.pallas_call(
        _kernel,
        grid=(B * H // 2 // _TH,),
        in_specs=[
            pl.BlockSpec((2 * _TH, W, C), lambda i: (i, 0, 0)),
            pl.BlockSpec((_TH, W // 2, C), lambda i: (i, 0, 0)),
            pl.BlockSpec((C, C), lambda i: (0, 0)),
            pl.BlockSpec((C, C), lambda i: (0, 0)),
        ],
        out_specs=pl.BlockSpec((2 * _TH, W, C), lambda i: (i, 0, 0)),
        out_shape=jax.ShapeDtypeStruct((B * H, W, C), c_fine.dtype),
        scratch_shapes=[pltpu.VMEM((C, C), jnp.bfloat16)],
        compiler_params=pltpu.CompilerParams(
            dimension_semantics=("arbitrary",), vmem_limit_bytes=100 * 1024 * 1024
        ),
    )(
        c_fine.reshape(B * H, W, C),
        p_coarse.reshape(B * H // 2, W // 2, C),
        w_lat,
        w_out.reshape(C, C),
    )
    return out.reshape(B, H, W, C)
```

```python
import jax
import jax.numpy as jnp
from jax import lax
import jax.experimental.pallas as pl
import jax.experimental.pallas.tpu as pltpu

_G = 8
_SR = 8
_RUN = 32
_TH = 4
_FIRST_WRITE_STEP = 19
_WRITE_BURST = 48
_WRITES_PER_STEP = 16
_READ_BOUNDS = (1, 2, 4, 7, 8, 10, 15)


def _upsample_rows(q):
    bits = pltpu.bitcast(q.astype(jnp.bfloat16).astype(jnp.float32), jnp.uint32)
    return pltpu.bitcast(bits | (bits >> 16), jnp.bfloat16).astype(jnp.float32)


@jax.jit
def pallas_standalone__detection_seg_fpn_lateral__vision_kernel(
    c_fine: jax.Array,
    p_coarse: jax.Array,
    w_lat: jax.Array,
    w_out: jax.Array,
):
    B, H, W, C = c_fine.shape
    n_bands = B * H // 2 // (_G * _SR)
    n_units = n_bands * _SR
    steps_per_unit = _G // _TH
    n_steps = n_units * steps_per_unit
    writes_per_unit = 2 * W // _RUN

    chunks = [
        ((0, pl.ds(k * _TH, _TH), pl.ds(0, 1)), k) for k in range(steps_per_unit)
    ]
    for u0, u1 in zip(_READ_BOUNDS[:-1], _READ_BOUNDS[1:]):
        box = (u0 // _SR, slice(None), pl.ds(u0 % _SR, u1 - u0))
        chunks.append((box, u0 * steps_per_unit))
    last = (n_units - 1) * steps_per_unit
    chunks.append(((n_bands - 1, pl.ds(0, _G - 1), pl.ds(_SR - 1, 1)), last))
    chunks.append(((n_bands - 1, pl.ds(_G - 1, 1), pl.ds(_SR - 1, 1)), last))

    def kernel(c_hbm, p_hbm, wl_hbm, wo_hbm, o_hbm, cbuf, pbuf, wl, wo, weff, sems):
        wsem = sems.at[len(chunks)]

        def reads(i):
            box = chunks[i][0]
            return (
                pltpu.make_async_copy(p_hbm.at[box], pbuf.at[box], sems.at[i]),
                pltpu.make_async_copy(c_hbm.at[box], cbuf.at[box], sems.at[i]),
            )

        def wait_reads(i):
            for d in reads(i):
                d.wait()

        weights = (
            pltpu.make_async_copy(wl_hbm, wl, wsem),
            pltpu.make_async_copy(wo_hbm, wo, wsem),
        )
        for d in weights:
            d.start(priority=1)
        for i in range(len(chunks)):
            for d in reads(i):
                d.start(priority=1)
        for d in weights:
            d.wait()
        weff[...] = jnp.dot(
            wl[...], wo[...], preferred_element_type=jnp.float32
        ).astype(weff.dtype)

        def write(w, _):
            u = w // writes_per_unit
            run = pl.ds(pl.multiple_of((w % writes_per_unit) * _RUN, _RUN), _RUN)
            box = (u // _SR, slice(None), u % _SR, run)
            pltpu.make_async_copy(cbuf.at[box], o_hbm.at[box], wsem).start(priority=1)

        def written_by(s):
            return jnp.minimum(
                writes_per_unit * (s // steps_per_unit),
                _WRITE_BURST + _WRITES_PER_STEP * (s - _FIRST_WRITE_STEP),
            )

        def step(s, _):
            for i, (_, need) in enumerate(chunks):
                if need < _FIRST_WRITE_STEP:
                    pl.when(s == need)(lambda i=i: wait_reads(i))

            @pl.when(s == _FIRST_WRITE_STEP)
            def _():
                for i, (_, need) in enumerate(chunks[:-1]):
                    if need >= _FIRST_WRITE_STEP:
                        wait_reads(i)
                lax.fori_loop(0, written_by(_FIRST_WRITE_STEP), write, None)
                wait_reads(len(chunks) - 1)

            @pl.when(s > _FIRST_WRITE_STEP)
            def _():
                lax.fori_loop(written_by(s - 1), written_by(s), write, None)

            u = s // steps_per_unit
            b, r = u // _SR, u % _SR
            for t in range(_TH):
                g = (s % steps_per_unit) * _TH + t
                q = jnp.dot(pbuf[b, g, r], wo[...], preferred_element_type=jnp.float32)
                up = _upsample_rows(q)
                for hh in range(2):
                    rows = pl.ds(hh * W, W)
                    a = jnp.dot(
                        cbuf[b, g, r, rows],
                        weff[...],
                        preferred_element_type=jnp.float32,
                    )
                    cbuf[b, g, r, rows] = (a + up).astype(cbuf.dtype)

        lax.fori_loop(0, n_steps, step, None)
        lax.fori_loop(written_by(n_steps - 1), n_units * writes_per_unit, write, None)
        pltpu.make_async_copy(cbuf, cbuf, wsem).wait()

    fine = (n_bands, _G, _SR, 2 * W, C)
    coarse = (n_bands, _G, _SR, W // 2, C)
    out = pl.pallas_call(
        kernel,
        in_specs=[pl.BlockSpec(memory_space=pl.ANY)] * 4,
        out_specs=pl.BlockSpec(memory_space=pl.ANY),
        out_shape=jax.ShapeDtypeStruct(fine, c_fine.dtype),
        scratch_shapes=[
            pltpu.VMEM(fine, c_fine.dtype),
            pltpu.VMEM(coarse, p_coarse.dtype),
            pltpu.VMEM((C, C), w_lat.dtype),
            pltpu.VMEM((C, C), w_out.dtype),
            pltpu.VMEM((C, C), c_fine.dtype),
            pltpu.SemaphoreType.DMA((len(chunks) + 1,)),
        ],
        compiler_params=pltpu.CompilerParams(vmem_limit_bytes=100 * 1024 * 1024),
    )(c_fine.reshape(fine), p_coarse.reshape(coarse), w_lat, w_out.reshape(C, C))
    return out.reshape(B, H, W, C)
```

```python
import jax
import jax.numpy as jnp
from jax import lax
import jax.experimental.pallas as pl
import jax.experimental.pallas.tpu as pltpu

_STREAMS = 8
_ROWS = 8
_STEP = 4
_SLOTS = 3 * _STEP

_READ_RUN = 16
_READ_PRIORITY = (1, 0, 1, 1, 0)
_READ_STEPS = 17
_READS_PER_STEP = 27

_WRITE_RUN = 32
_FIRST_WRITE_SLOT = 5


def _divmod(x, n):
    assert n & (n - 1) == 0
    return lax.shift_right_logical(x, n.bit_length() - 1), x & (n - 1)


def _repeat_rows(q):
    bits = pltpu.bitcast(q.astype(jnp.bfloat16).astype(jnp.float32), jnp.uint32)
    return pltpu.bitcast(bits | (bits >> 16), jnp.bfloat16).astype(jnp.float32)


@jax.jit
def pallas_standalone__detection_seg_fpn_lateral__vision_kernel(
    c_fine: jax.Array,
    p_coarse: jax.Array,
    w_lat: jax.Array,
    w_out: jax.Array,
):
    B, H, W, C = c_fine.shape
    dtype = c_fine.dtype
    assert dtype == jnp.bfloat16 and w_out.shape == (1, 1, C, C)
    assert p_coarse.shape == (B, H // 2, W // 2, C)
    assert (B * H) % (2 * _STREAMS * _ROWS) == 0

    n_bands = B * H // (2 * _STREAMS * _ROWS)
    n_units = n_bands * _ROWS
    steps_per_unit = _STREAMS // _STEP
    n_steps = n_units * steps_per_unit
    reads_per_unit = 2 * W // _READ_RUN
    writes_per_unit = 2 * W // _WRITE_RUN
    reads_up_front = n_units * reads_per_unit - _READ_STEPS * _READS_PER_STEP
    for s in range(n_steps):
        done = s // steps_per_unit
        if s < _READ_STEPS:
            assert (done + 1) * reads_per_unit <= reads_up_front + s * _READS_PER_STEP
        else:
            assert s - _READ_STEPS < done

    def kernel(c_hbm, p_hbm, wl_hbm, wo_hbm, o_hbm, x_buf, o_buf, w_buf, w_eff, o_sem):
        def body(sems):
            def read(i):
                unit, col = _divmod(i, reads_per_unit)
                band, row = _divmod(unit, _ROWS)
                quarter = _STREAMS // 4
                p_col, p_part = _divmod(col, 4)
                streams = pl.ds(p_part * quarter, quarter)
                start = pl.multiple_of(p_col * _READ_RUN, _READ_RUN)
                pltpu.make_async_copy(
                    p_hbm.at[band, streams, row, pl.ds(start, _READ_RUN)],
                    x_buf.at[band, streams, row, pl.ds(start + 2 * W, _READ_RUN)],
                    sems.at[unit],
                ).start(priority=_READ_PRIORITY[0])
                start = pl.multiple_of(col * _READ_RUN, _READ_RUN)
                for part in range(4):
                    streams = pl.ds(part * quarter, quarter)
                    box = (band, streams, row, pl.ds(start, _READ_RUN))
                    pltpu.make_async_copy(
                        c_hbm.at[box], x_buf.at[box], sems.at[unit]
                    ).start(priority=_READ_PRIORITY[1 + part])

            def write(i):
                unit, col = _divmod(i, writes_per_unit)
                band, row = _divmod(unit, _ROWS)
                start = pl.multiple_of(col * _WRITE_RUN, _WRITE_RUN)
                box = (band, slice(None), row, pl.ds(start, _WRITE_RUN))
                pltpu.make_async_copy(o_buf.at[box], o_hbm.at[box], o_sem).start()

            def step(s, issue, first, count, first_slot):
                unit, part = _divmod(s, steps_per_unit)
                band, row = _divmod(unit, _ROWS)

                @pl.when(part == 0)
                def _():
                    dst = x_buf.at[band, :, row]
                    pltpu.make_async_copy(dst, dst, sems.at[unit]).wait()

                def issue_share(slot):
                    k, n = slot - first_slot, _SLOTS - first_slot
                    if k >= 0:
                        for i in range(count * k // n, count * (k + 1) // n):
                            issue(first + i)

                for t in range(_STEP):
                    stream = part * _STEP + t
                    issue_share(3 * t)
                    top_down = _repeat_rows(
                        jnp.dot(
                            x_buf[band, stream, row, pl.ds(2 * W, W // 2)],
                            w_buf[1],
                            preferred_element_type=jnp.float32,
                        )
                    )
                    for h in range(2):
                        issue_share(3 * t + 1 + h)
                        pixels = pl.ds(h * W, W)
                        lateral = jnp.dot(
                            x_buf[band, stream, row, pixels],
                            w_eff[...],
                            preferred_element_type=jnp.float32,
                        )
                        o_buf[band, stream, row, pixels] = (lateral + top_down).astype(
                            dtype
                        )

            w_sem = sems.at[n_units]
            pltpu.make_async_copy(wl_hbm, w_buf.at[0], w_sem).start(priority=1)
            pltpu.make_async_copy(wo_hbm, w_buf.at[1], w_sem).start(priority=1)
            lax.fori_loop(0, reads_up_front, lambda i, _: read(i), None)
            pltpu.make_async_copy(w_buf, w_buf, w_sem).wait()
            w_eff[...] = jnp.dot(
                w_buf[0], w_buf[1], preferred_element_type=jnp.float32
            ).astype(dtype)

            def read_step(s, _):
                first = reads_up_front + s * _READS_PER_STEP
                step(s, read, first, _READS_PER_STEP, 0)

            def write_step(s, _):
                first = (s - _READ_STEPS) * writes_per_unit
                step(s, write, first, writes_per_unit, _FIRST_WRITE_SLOT)

            lax.fori_loop(0, _READ_STEPS, read_step, None)
            lax.fori_loop(_READ_STEPS, n_steps, write_step, None)
            lax.fori_loop(
                (n_steps - _READ_STEPS) * writes_per_unit,
                n_units * writes_per_unit,
                lambda i, _: write(i),
                None,
            )

        pl.run_scoped(body, pltpu.SemaphoreType.DMA((n_units + 1,)))
        pltpu.make_async_copy(o_buf, o_buf, o_sem).wait()

    lead = (n_bands, _STREAMS, _ROWS)
    out = pl.pallas_call(
        kernel,
        in_specs=[pl.BlockSpec(memory_space=pl.ANY)] * 4,
        out_specs=pl.BlockSpec(memory_space=pl.ANY),
        out_shape=jax.ShapeDtypeStruct(lead + (2 * W, C), dtype),
        scratch_shapes=[
            pltpu.VMEM(lead + (2 * W + W // 2, C), dtype),
            pltpu.VMEM(lead + (2 * W, C), dtype),
            pltpu.VMEM((2, C, C), dtype),
            pltpu.VMEM((C, C), dtype),
            pltpu.SemaphoreType.DMA(()),
        ],
        compiler_params=pltpu.CompilerParams(vmem_limit_bytes=120 * 1024 * 1024),
    )(
        c_fine.reshape(lead + (2 * W, C)),
        p_coarse.reshape(lead + (W // 2, C)),
        w_lat,
        w_out.reshape(C, C),
    )
    return out.reshape(B, H, W, C)
```
